```python
import os as _os
_os.environ.setdefault("JAX_PLATFORMS", "cpu")
import jax
import jax.numpy as jnp

def _softmax(x, axis=-1):
    return jax.nn.softmax(x, axis=axis)
def _gelu(x):
    return jax.nn.gelu(x, approximate=True)
def _silu(x):
    return jax.nn.silu(x)
def _sigmoid(x):
    return jax.nn.sigmoid(x)
def _layernorm(x, axis=-1, eps=1e-5):
    m = jnp.mean(x, axis=axis, keepdims=True)
    v = jnp.var(x, axis=axis, keepdims=True)
    return (x - m) / jnp.sqrt(v + eps)
def _scatter_add(tgt, idx, src, axis=0):
    return tgt.at[idx].add(src)
def _segment_sum(src, seg, n):
    return jax.ops.segment_sum(src, seg, n)
class _Rng:
    def __init__(self, key):
        self._k = key
    def _next(self):
        self._k, sub = jax.random.split(self._k)
        return sub
    def normal(self, shape):
        return jax.random.normal(self._next(), shape, dtype=jnp.bfloat16)
    def randint(self, lo, hi, shape):
        return jax.random.randint(self._next(), shape, lo, hi, dtype=jnp.int32)
    def uniform(self, shape, lo=0.0, hi=1.0):
        return jax.random.uniform(self._next(), shape, jnp.bfloat16, lo, hi)
    def permutation(self, n):
        return jax.random.permutation(self._next(), n)


kernel_name = 'gated_mix__sliding_block_cached__swiglu_ffn__decode'

def setup_inputs():
    _rng = _Rng(jax.random.key(int.from_bytes(__import__("os").urandom(4), "little")))
    _w = (lambda a: (lambda t: t.astype(jnp.bfloat16) if jnp.issubdtype(t.dtype, jnp.floating) else t)(jnp.asarray(a)))
    def _A_setup():
        B, Sq, D = 1, 1, 512
        Hq, Hkv, Sk, Dh = 32, 32, 32768, 128
        assert Hq % Hkv == 0, (Hq, Hkv)
        return {
            "x": _w((lambda *s: _rng.normal(s) * 0.05)(B, Sq, D)),
            "k_cache": _w((lambda *s: _rng.normal(s) * 3.2)(B, Hkv, Sk, Dh)),
            "v_cache": _w((lambda *s: _rng.normal(s) * 1.6)(B, Hkv, Sk, Dh)),
            "wq": _w((lambda *s: _rng.normal(s) * 3.2)(D, Hq * Dh) * (D ** -0.5)),
            "wo": _w((lambda *s: _rng.normal(s) * 1.6)(Hq * Dh, D) * ((Hq * Dh) ** -0.5)),
        }
    _A_in = _A_setup()

    def _B_setup():
        B, S, D, F = 1, 1, 512, 1376
        return {
            "x": _w((lambda *s: _rng.normal(s) * 0.05)(B, S, D)),
            "w_gate": _w((lambda *s: _rng.normal(s) * 0.1)(D, F)),
            "w_up": _w((lambda *s: _rng.normal(s) * 0.1)(D, F)),
            "w_down": _w((lambda *s: _rng.normal(s) * 0.1)(F, D)),
        }
    _B_in = _B_setup()

    return {
        "A_x": _A_in["x"],
        "A_k_cache": _A_in["k_cache"],
        "A_v_cache": _A_in["v_cache"],
        "A_wq": _A_in["wq"],
        "A_wo": _A_in["wo"],
        "B_x": _B_in["x"],
        "B_w_gate": _B_in["w_gate"],
        "B_w_up": _B_in["w_up"],
        "B_w_down": _B_in["w_down"],
        "gate_w": _w((lambda *s: _rng.normal(s) * 0.05)(512) * 16.0),
    }

def reference(A_x, A_k_cache, A_v_cache, A_wq, A_wo, B_x, B_w_gate, B_w_up, B_w_down, gate_w):
    def _A_ref(x, k_cache, v_cache, wq, wo):
        B, Sq, D = x.shape
        Hq, Dh = 32, 128
        Hkv, Sk = k_cache.shape[1], k_cache.shape[2]
        W = min(4096, max(256, Sk // 4))
        rep = Hq // Hkv
        q = (lambda x, *d: x.transpose(*d))((x @ wq).reshape(B, Sq, Hq, Dh), 0, 2, 1, 3)
        k = jnp.repeat(k_cache[:, :, Sk - W:, :], rep, axis=1)
        v = jnp.repeat(v_cache[:, :, Sk - W:, :], rep, axis=1)
        scores = jnp.einsum("bhqd,bhkd->bhqk", q, k) * (Dh ** -0.5)
        p = _softmax(scores, axis=-1)
        o = jnp.einsum("bhqk,bhkd->bhqd", p, v)
        return (lambda x, *d: x.transpose(*d))(o, 0, 2, 1, 3).reshape(B, Sq, Hq * Dh) @ wo

    def _B_ref(x, w_gate, w_up, w_down):
        g = _silu(x @ w_gate)
        u = x @ w_up
        return (g * u) @ w_down

    x = A_x
    g = _sigmoid((x * gate_w).sum(-1, keepdims=True))
    a = _A_ref(x, A_k_cache, A_v_cache, A_wq, A_wo)
    b = _B_ref(x, B_w_gate, B_w_up, B_w_down)
    return g * a + (1 - g) * b
```

```python
import jax
import jax.numpy as jnp
from jax import lax
import jax.experimental.pallas as pl
import jax.experimental.pallas.tpu as pltpu

_HQ, _DH = 32, 128
_NT = (((1,), (1,)), ((), ()))
_NN = (((1,), (0,)), ((), ()))
_NBUF = 2


def _dot(a, b, dims):
    return lax.dot_general(a, b, dims, preferred_element_type=jnp.float32)


@jax.jit
def pallas_gated_mix__sliding_block_cached__swiglu_ffn__decode_kernel(
    A_x: jax.Array,
    A_k_cache: jax.Array,
    A_v_cache: jax.Array,
    A_wq: jax.Array,
    A_wo: jax.Array,
    B_x: jax.Array,
    B_w_gate: jax.Array,
    B_w_up: jax.Array,
    B_w_down: jax.Array,
    gate_w: jax.Array,
):
    del B_x
    D = A_x.shape[-1]
    SK = A_k_cache.shape[2]
    W = min(4096, max(256, SK // 4))
    F = B_w_gate.shape[1]
    bf = A_x.dtype
    scale = _DH ** -0.5
    nbuf = _NBUF

    def kernel(x_hbm, k_hbm, v_hbm, wq_hbm, wo_hbm, wg_hbm, wu_hbm, wd_hbm, gw_hbm, o_ref,
               x_v, gw_v, wq_v, wo_v, wg_v, wu_v, wd_v, k_v, v_v, sem, ksem, vsem):
        def kcopy(h, slot):
            return pltpu.make_async_copy(k_hbm.at[0, h, pl.ds(SK - W, W), :], k_v.at[slot], ksem.at[slot])

        def vcopy(h, slot):
            return pltpu.make_async_copy(v_hbm.at[0, h, pl.ds(SK - W, W), :], v_v.at[slot], vsem.at[slot])

        small = [pltpu.make_async_copy(s, d, sem.at[i]) for i, (s, d) in enumerate(
            [(x_hbm, x_v), (gw_hbm, gw_v), (wg_hbm, wg_v), (wu_hbm, wu_v), (wd_hbm, wd_v),
             (wq_hbm, wq_v), (wo_hbm, wo_v)])]
        for c in small:
            c.start()
        for h in range(nbuf):
            kcopy(h, h).start()
            vcopy(h, h).start()
        small[0].wait()
        small[1].wait()
        x1 = x_v[0]
        x8 = jnp.broadcast_to(x1, (8, D))
        gw = gw_v[...].astype(jnp.float32)
        xf = x1.astype(jnp.float32)
        prod = sum(xf[:, i * 128:(i + 1) * 128] * gw[i:i + 1, :] for i in range(D // 128))
        gate = jax.nn.sigmoid(jnp.sum(prod, axis=-1, keepdims=True))
        small[2].wait()
        g = _dot(x8, wg_v[...], _NT)
        small[3].wait()
        u = _dot(x8, wu_v[...], _NT)
        hid = (g * jax.nn.sigmoid(g) * u).astype(bf)
        small[4].wait()
        b = _dot(hid, wd_v[...], _NN)
        small[5].wait()
        small[6].wait()

        def body(h, acc):
            slot = h % nbuf
            off = pl.multiple_of(h * _DH, _DH)
            q = _dot(x8, wq_v[:, pl.ds(off, _DH)], _NN).astype(bf)
            kcopy(h, slot).wait()
            s = _dot(q, k_v[slot], _NT) * scale
            m = jnp.max(s, axis=-1, keepdims=True)
            p = jnp.exp(s - m)
            l = jnp.sum(p, axis=-1, keepdims=True)

            @pl.when(h + nbuf < _HQ)
            def _():
                kcopy(h + nbuf, slot).start()

            vcopy(h, slot).wait()
            o = _dot(p.astype(bf), v_v[slot], _NN) / l

            @pl.when(h + nbuf < _HQ)
            def _():
                vcopy(h + nbuf, slot).start()

            return acc + _dot(o.astype(bf), wo_v[pl.ds(off, _DH), :], _NN)

        a = lax.fori_loop(0, _HQ, body, jnp.zeros((8, D), jnp.float32))
        res = gate * a[0:1] + (1.0 - gate) * b[0:1]
        o_ref[0] = res.astype(o_ref.dtype)

    hbm = pl.BlockSpec(memory_space=pltpu.HBM)
    return pl.pallas_call(
        kernel,
        out_shape=jax.ShapeDtypeStruct(A_x.shape, bf),
        in_specs=[hbm] * 9,
        scratch_shapes=[
            pltpu.VMEM(A_x.shape, bf), pltpu.VMEM((D // 128, 128), bf),
            pltpu.VMEM(A_wq.shape, bf), pltpu.VMEM(A_wo.shape, bf),
            pltpu.VMEM((F, D), bf), pltpu.VMEM((F, D), bf), pltpu.VMEM((F, D), bf),
            pltpu.VMEM((nbuf, W, _DH), bf), pltpu.VMEM((nbuf, W, _DH), bf),
            pltpu.SemaphoreType.DMA((7,)), pltpu.SemaphoreType.DMA((nbuf,)),
            pltpu.SemaphoreType.DMA((nbuf,)),
        ],
        compiler_params=pltpu.CompilerParams(vmem_limit_bytes=100 * 2**20),
    )(A_x, A_k_cache, A_v_cache, A_wq, A_wo, B_w_gate.T, B_w_up.T, B_w_down,
      gate_w.reshape(D // 128, 128))
```

```python
import functools
import jax
import jax.numpy as jnp
from jax import lax
import jax.experimental.pallas as pl
import jax.experimental.pallas.tpu as pltpu

HQ, DH = 32, 128
NT = (((1,), (1,)), ((), ()))
NN = (((1,), (0,)), ((), ()))
f32 = jnp.float32

def _dot(a, b, dims):
    return lax.dot_general(a, b, dims, preferred_element_type=f32)

def make(depth=8, hi=2, cyc=True, whi=32, checks=False, p_hi=0, p_lo=1):
  def fn(A_x, A_k_cache, A_v_cache, A_wq, A_wo, B_x, B_w_gate, B_w_up, B_w_down, gate_w):
    del B_x
    D = A_x.shape[-1]
    SK = A_k_cache.shape[2]
    W = min(4096, max(256, SK // 4))
    F = B_w_gate.shape[1]
    bf = A_x.dtype
    scale = DH ** -0.5
    G = HQ // 8
    NC = W // 128
    NB = G * NC
    R = 16
    assert depth // 2 + 2 <= R
    KC = D // 128
    NQ = KC * (HQ // 4)
    FC = F // 128
    FR = F - FC * 128

    def kernel(x_hbm, k_hbm, v_hbm, wq_hbm, wo_hbm, wg_hbm, wu_hbm, wd_hbm, gw_hbm, o_ref,
               x_v, gw_v, wq_v, wo_v, wg_v, wu_v, wd_v, kv_v, xs_v, q_v, s_v, m_v, l_v, acc_v, sem, xsem):
        row = lax.broadcasted_iota(jnp.int32, (8, 128), 0)

        def slot(g):
            return g % depth if isinstance(g, int) else lax.rem(g, depth)

        def start2(src, dst, n_hi, n, g):
            pltpu.make_async_copy(src.at[pl.ds(n_hi, n - n_hi)], dst.at[pl.ds(n_hi, n - n_hi)], sem.at[slot(g)]).start(priority=p_lo)
            pltpu.make_async_copy(src.at[pl.ds(0, n_hi)], dst.at[pl.ds(0, n_hi)], sem.at[slot(g)]).start(priority=p_hi)
        def wait(dst, g):
            pltpu.make_async_copy(dst, dst, sem.at[slot(g)]).wait()

        def wq_view(ref, s):
            kc, hc = s % KC, s // KC
            return ref.at[pl.ds(pl.multiple_of(kc * 128, 128), 128), pl.ds(pl.multiple_of(hc * 512, 512), 512)]
        def rows_view(ref, c, n=128):
            return ref.at[pl.ds(pl.multiple_of(c * 128, 128), n)]
        def blk(t):
            return (t % G, t // G) if cyc else (t // NC, t % NC)
        def kv_src(ref, s):
            g, c = blk(s // 2)
            return ref.at[g, :, pl.ds(pl.multiple_of(SK - W + c * 128 + (s % 2) * 64, 64), 64)]
        def kv_dst(s):
            return kv_v.at[(s // 2) % R, :, pl.ds(pl.multiple_of((s % 2) * 64, 64), 64)]

        ffn = ((wg_hbm, wg_v), (wu_hbm, wu_v), (wd_hbm, wd_v))
        g_q, g_f = 0, NQ
        NF = 3 * (FC + 1)
        g_k = g_f + NF
        g_v = g_k + 2 * NB
        g_o = g_v + 2 * NB

        def issue_q(s): start2(wq_view(wq_hbm, s), wq_view(wq_v, s), whi, 128, g_q + s)
        def issue_f(c, j, n=128): start2(rows_view(ffn[j][0], c, n), rows_view(ffn[j][1], c, n), whi, n, g_f + 3 * c + j)
        def issue_k(s): start2(kv_src(k_hbm, s), kv_dst(s), hi, 8, g_k + s)
        def issue_v(s): start2(kv_src(v_hbm, s), kv_dst(s), hi, 8, g_v + s)
        def issue_o(s): start2(rows_view(wo_hbm, s), rows_view(wo_v, s), whi, 128, g_o + s)
        def issue_f_static(s):
            if s < NF:
                c, j = divmod(s, 3)
                issue_f(c, j, 128 if c < FC else FR)
            else:
                issue_k(s - NF)

        cx = pltpu.make_async_copy(x_hbm, x_v, xsem.at[0])
        cg = pltpu.make_async_copy(gw_hbm, gw_v, xsem.at[0])
        cx.start(); cg.start()
        for s in range(depth):
            issue_q(s)
        cx.wait(); cg.wait()
        x1 = x_v[0]
        xf = x1.astype(f32)
        gw = gw_v[...].astype(f32)
        prod = sum(xf[:, i*128:(i+1)*128] * gw[i:i+1, :] for i in range(KC))
        gate = jax.nn.sigmoid(jnp.sum(prod, axis=-1, keepdims=True))
        for i in range(KC):
            xs_v[i] = jnp.broadcast_to(xf[:, i*128:(i+1)*128], (8, 128))
        q_v[...] = jnp.zeros(q_v.shape, f32)
        m_v[...] = jnp.full(m_v.shape, -jnp.inf, f32)
        l_v[...] = jnp.zeros(l_v.shape, f32)
        acc_v[...] = jnp.zeros(acc_v.shape, f32)

        def q_compute(s):
            kc, hc = s % KC, s // KC
            r = _dot(xs_v[kc].astype(bf), wq_view(wq_v, s)[...], NN)
            base = (hc % 2) * 4
            upd = jnp.zeros((8, 128), f32)
            for j in range(4):
                upd = jnp.where(row == base + j, r[:, j*128:(j+1)*128], upd)
            q_v[hc // 2] += upd
        def q_body(s, _):
            wait(wq_view(wq_v, s), g_q + s)
            issue_q(s + depth)
            q_compute(s)
        lax.fori_loop(0, NQ - depth, q_body, None)
        def q_body2(s, _):
            wait(wq_view(wq_v, s), g_q + s)
            n = s + depth - NQ
            for j in range(3):
                @pl.when(n % 3 == j)
                def _(): issue_f(n // 3, j)
            q_compute(s)
        lax.fori_loop(NQ - depth, NQ, q_body2, None)

        x8 = jnp.broadcast_to(x1, (8, D))
        def f_step(c, j, n, issue):
            wait(rows_view(ffn[j][1], c, n), g_f + 3 * c + j)
            issue(j)
            return rows_view(ffn[j][1], c, n)[...]
        def f_body(c, b, n=128, issue=None):
            g = _dot(x8, f_step(c, 0, n, issue), NT)
            u = _dot(x8, f_step(c, 1, n, issue), NT)
            h = (g * jax.nn.sigmoid(g) * u).astype(bf)
            return b + _dot(h, f_step(c, 2, n, issue), NN)
        def f_dyn(c, b):
            def issue(j):
                dc, jj = divmod(j + depth, 3)
                cc = c + dc
                @pl.when(cc < FC)
                def _(): issue_f(cc, jj)
                @pl.when(cc == FC)
                def _(): issue_f(FC, jj, FR)
                @pl.when(cc > FC)
                def _(): issue_k(3 * cc + jj - NF)
            return f_body(c, b, 128, issue)
        b = lax.fori_loop(0, FC, f_dyn, jnp.zeros((8, D), f32))
        b = f_body(FC, b, FR, lambda j: issue_f_static(3 * FC + j + depth))

        def advance(s, g0, own, nxt):
            wait(kv_dst(s), g0 + s)
            @pl.when(s + depth < 2 * NB)
            def _(): own(s + depth)
            @pl.when(s + depth >= 2 * NB)
            def _(): nxt(s + depth - 2 * NB)
        def k_body(t, _):
            advance(2 * t, g_k, issue_k, issue_v)
            advance(2 * t + 1, g_k, issue_k, issue_v)
            g, c = blk(t)
            q8 = q_v[g].astype(bf)
            s8 = None
            for j in range(8):
                r = _dot(q8, kv_v[t % R, j], NT)
                s8 = r if s8 is None else jnp.where(row == j, r, s8)
            s8 = s8 * scale
            s_v[t] = s8
            m_v[g] = jnp.maximum(m_v[g], s8)
        lax.fori_loop(0, NB, k_body, None)
        m_all = m_v[...]
        m_v[...] = jnp.broadcast_to(jnp.max(m_all, axis=-1, keepdims=True), m_all.shape)

        def v_body(t, _):
            advance(2 * t, g_v, issue_v, issue_o)
            advance(2 * t + 1, g_v, issue_v, issue_o)
            g, c = blk(t)
            p = jnp.exp(s_v[t] - m_v[g])
            l_v[g] += p
            pb = p.astype(bf)
            o8 = None
            for j in range(8):
                r = _dot(pb, kv_v[t % R, j], NN)
                o8 = r if o8 is None else jnp.where(row == j, r, o8)
            acc_v[g] += o8
        lax.fori_loop(0, NB, v_body, None)
        acc_v[...] = acc_v[...] / jnp.sum(l_v[...], axis=-1, keepdims=True)

        def o_body(h, a):
            wait(rows_view(wo_v, h), g_o + h)
            @pl.when(h + depth < HQ)
            def _(): issue_o(h + depth)
            oh = jnp.where(row == h % 8, acc_v[h // 8], 0.0).astype(bf)
            return a + _dot(oh, rows_view(wo_v, h)[...], NN)
        a = lax.fori_loop(0, HQ, o_body, jnp.zeros((8, D), f32))
        a1 = jnp.sum(a, axis=0, keepdims=True)
        res = gate * a1 + (1.0 - gate) * b[0:1]
        o_ref[0] = res.astype(o_ref.dtype)

    HBM = pl.BlockSpec(memory_space=pltpu.HBM)
    return pl.pallas_call(
        kernel,
        out_shape=jax.ShapeDtypeStruct(A_x.shape, bf),
        in_specs=[HBM] * 9,
        scratch_shapes=[
            pltpu.VMEM(A_x.shape, bf), pltpu.VMEM((D // 128, 128), bf),
            pltpu.VMEM(A_wq.shape, bf), pltpu.VMEM(A_wo.shape, bf),
            pltpu.VMEM((F, D), bf), pltpu.VMEM((F, D), bf), pltpu.VMEM((F, D), bf),
            pltpu.VMEM((R, 8, 128, DH), bf),
            pltpu.VMEM((KC, 8, 128), f32), pltpu.VMEM((G, 8, 128), f32), pltpu.VMEM((NB, 8, 128), f32),
            pltpu.VMEM((G, 8, 128), f32), pltpu.VMEM((G, 8, 128), f32), pltpu.VMEM((G, 8, 128), f32),
            pltpu.SemaphoreType.DMA((depth,)), pltpu.SemaphoreType.DMA((1,)),
        ],
        compiler_params=pltpu.CompilerParams(vmem_limit_bytes=64 * 2**20, disable_bounds_checks=not checks,
                                             disable_semaphore_checks=not checks),
    )(A_x, A_k_cache.reshape(G, 8, SK, DH), A_v_cache.reshape(G, 8, SK, DH), A_wq, A_wo,
      B_w_gate.T, B_w_up.T, B_w_down, gate_w.reshape(D // 128, 128))
  return fn


_impl = make(checks=True)


@jax.jit
def pallas_gated_mix__sliding_block_cached__swiglu_ffn__decode_kernel(
    A_x, A_k_cache, A_v_cache, A_wq, A_wo, B_x, B_w_gate, B_w_up, B_w_down, gate_w):
    return _impl(A_x, A_k_cache, A_v_cache, A_wq, A_wo, B_x, B_w_gate, B_w_up, B_w_down, gate_w)
```

```python
import functools

import jax
import jax.numpy as jnp
from jax import lax
import jax.experimental.pallas as pl
import jax.experimental.pallas.tpu as pltpu

_HQ, _DH = 32, 128
_NT = (((1,), (1,)), ((), ()))
_NN = (((1,), (0,)), ((), ()))
_HI, _LO = 0, 1
_FAR, _NEAR = 10, 7
_NSEM = 16
_RING = 16


def _dot(a, b, dims):
    return lax.dot_general(a, b, dims, preferred_element_type=jnp.float32)


def _div(a, n):
    assert n & (n - 1) == 0
    return a // n if isinstance(a, int) else lax.shift_right_logical(a, n.bit_length() - 1)


def _mod(a, n):
    assert n & (n - 1) == 0
    return a & (n - 1)


def _ds(start, size, align=None):
    if isinstance(start, int):
        return pl.ds(start, size)
    return pl.ds(pl.multiple_of(start, align or size), size)


def _kernel(x_hbm, k_hbm, v_hbm, wq_hbm, wo_hbm, wg_hbm, wu_hbm, wd_hbm, gw_hbm, o_ref,
            x_v, gw_v, wq_v, wo_v, wg_v, wu_v, wd_v, kv_v, q_v, s_v, m_v, l_v, acc_v,
            sems, xsem, *, window):
    f32 = jnp.float32
    dtype = x_v.dtype
    d_model = x_v.shape[-1]
    n_groups, _, seq, _ = k_hbm.shape
    n_chunks = window // 128
    n_blocks = n_groups * n_chunks
    f_half = wg_v.shape[1]
    f_chunks = pl.cdiv(f_half, 128)
    row = lax.broadcasted_iota(jnp.int32, (8, 128), 0)
    lane = lax.broadcasted_iota(jnp.int32, (8, 128), 1)

    def split(src, dst, n_hi):
        hi, lo = pl.ds(0, n_hi), pl.ds(n_hi, dst.shape[0] - n_hi)
        return {_HI: [(src.at[hi], dst.at[hi])], _LO: [(src.at[lo], dst.at[lo])]}

    def wq_step(s):
        view = lambda r: r.at[:, _ds(_div(s, 4) * 8, 8), _ds(_mod(s, 4) * 1024, 1024)]
        return split(view(wq_hbm), view(wq_v), 2)

    def ffn_step(s):
        pair = lambda src, dst: (src.at[:, _ds(s * 16, 16)], dst.at[:, _ds(s * 16, 16)])
        return {_HI: [pair(wg_hbm, wg_v)], _LO: [pair(wu_hbm, wu_v), pair(wd_hbm, wd_v)]}

    def group_of(t):
        return _div(t, 2 * n_chunks) * 2 + _mod(t, 2)

    def kv_step(ref, s):
        t, half = _div(s, 4) * 2 + _mod(s, 2), _mod(_div(s, 2), 2)
        key = seq - window + _mod(_div(t, 2), n_chunks) * 128 + half * 64
        return split(ref.at[group_of(t), :, _ds(key, 64)],
                     kv_v.at[_mod(t, _RING), :, _ds(half * 64, 64)], 2)

    def wo_step(s):
        view = lambda r: r.at[:, _ds(s * 16, 16)]
        return split(view(wo_hbm), view(wo_v), 2)

    def wo_last_step(s):
        view = lambda r: r.at[s, pl.ds(3 * _DH, _DH)]
        return split(view(wo_hbm), view(wo_v), 32)

    phases = [
        (32, wq_step),
        (f_half // 16, ffn_step),
        (2 * n_blocks, functools.partial(kv_step, k_hbm)),
        (24, wo_step),
        (2 * n_blocks, functools.partial(kv_step, v_hbm)),
        (8, wo_last_step),
    ]
    WQ, FFN, KEYS, WO, VALUES, WO_LAST = range(len(phases))
    first = [sum(n for n, _ in phases[:p]) for p in range(len(phases))]

    def copies(p, s, part):
        sem = sems.at[_mod(first[p] + s, _NSEM)]
        return [pltpu.make_async_copy(src, dst, sem) for src, dst in phases[p][1](s)[part]]

    def start(p, s, part, priority=None):
        for c in copies(p, s, part):
            c.start(priority=part if priority is None else priority)

    def advance(p, s):
        for c in copies(p, s, _HI) + copies(p, s, _LO):
            c.wait()
        for ahead, part in ((_FAR, _LO), (_NEAR, _HI)):
            for nxt in range(p, len(phases)):
                off = ahead + first[p] - first[nxt]
                n = phases[nxt][0]
                if off >= n or off + phases[p][0] <= 0:
                    continue
                if isinstance(s, int):
                    if 0 <= s + off < n:
                        start(nxt, s + off, part)
                    continue
                valid = []
                if off < 0:
                    valid.append(s + off >= 0)
                if off + phases[p][0] > n:
                    valid.append(s + off < n)
                pl.when(functools.reduce(jnp.logical_and, valid))(
                    functools.partial(start, nxt, s + off, part))

    def kv_loop(p, t0, n, compute):
        advance(p, 2 * t0)

        def body(i, _):
            t = t0 + i
            advance(p, 2 * t + 1)
            pl.when(i < n - 1)(lambda: advance(p, 2 * t + 2))
            compute(t)

        lax.fori_loop(0, n, body, None)

    def per_head(lhs, t, dims):
        out = _dot(lhs, kv_v[_mod(t, _RING), 0], dims)
        for j in range(1, 8):
            out = jnp.where(row == j, _dot(lhs, kv_v[_mod(t, _RING), j], dims), out)
        return out

    for s in range(_FAR):
        start(WQ, s, _LO)
        if s < _NEAR:
            start(WQ, s, _HI, priority=_LO)
    x_copy = pltpu.make_async_copy(x_hbm, x_v, xsem.at[0])
    gw_copy = pltpu.make_async_copy(gw_hbm, gw_v, xsem.at[0])
    x_copy.start()
    gw_copy.start()
    q_v[...] = jnp.zeros(q_v.shape, f32)
    m_v[...] = jnp.full(m_v.shape, -jnp.inf, f32)
    l_v[...] = jnp.zeros(l_v.shape, f32)
    acc_v[...] = jnp.zeros(acc_v.shape, f32)

    lax.fori_loop(0, phases[WQ][0], lambda s, _: advance(WQ, s), None)
    x_copy.wait()
    gw_copy.wait()
    x1 = x_v[0]
    x8 = jnp.broadcast_to(x1, (8, d_model))

    def q_body(i, _):
        advance(FFN, 2 * i)
        advance(FFN, 2 * i + 1)
        q2 = _dot(x8, wq_v[:, :, _ds(i * 2 * _DH, 2 * _DH)].reshape(d_model, 2 * _DH), _NN)
        g, j = _div(i, 4), _mod(i, 4) * 2
        q_v[g] = jnp.where(row == j, q2[:, :_DH], jnp.where(row == j + 1, q2[:, _DH:], q_v[g]))

    lax.fori_loop(0, _HQ // 2, q_body, None)
    xf, gw = x1.astype(f32), gw_v[...].astype(f32)
    prod = sum(xf[:, i * 128:(i + 1) * 128] * gw[i:i + 1] for i in range(d_model // 128))
    gate = jax.nn.sigmoid(jnp.sum(prod, axis=-1, keepdims=True))
    lax.fori_loop(_HQ, phases[FFN][0], lambda s, _: advance(FFN, s), None)

    def scores(t):
        g = group_of(t)
        s8 = per_head(q_v[g].astype(dtype), t, _NT) * (_DH ** -0.5)
        s_v[t] = s8
        m_v[g] = jnp.maximum(m_v[g], s8)

    kv_loop(KEYS, 0, n_blocks, scores)
    m_v[...] = jnp.broadcast_to(jnp.max(m_v[...], axis=-1, keepdims=True), m_v.shape)

    def ffn_body(i, b):
        half, c = _mod(i, 2), _div(i, 2)
        lo = jnp.minimum(c * 128, f_half - 128)
        rows = _ds(lo, 128, 16)
        advance(WO, 2 * i)
        g = _dot(x8, wg_v[half, rows], _NT)
        u = _dot(x8, wu_v[half, rows], _NT)
        advance(WO, 2 * i + 1)
        h = jnp.where(lane >= c * 128 - lo, g * jax.nn.sigmoid(g) * u, 0.0)
        return b + _dot(h.astype(dtype), wd_v[half, rows], _NN)

    assert 4 * f_chunks == phases[WO][0]
    b = lax.fori_loop(0, 2 * f_chunks, ffn_body, jnp.zeros((8, d_model), f32))
    b = (1.0 - gate) * b[0:1]

    def weigh_values(t):
        g = group_of(t)
        p = jnp.exp(s_v[t] - m_v[g])
        l_v[g] += p
        acc_v[g] += per_head(p.astype(dtype), t, _NN)

    def head_out(slab, i):
        return acc_v[_div(slab, 2), pl.ds(_mod(slab, 2) * 4 + i, 1)]

    def project(slab, i):
        o8 = jnp.broadcast_to(head_out(slab, i), (8, _DH)).astype(dtype)
        return _dot(o8, wo_v[slab, pl.ds(i * _DH, _DH)], _NN)

    def pair_body(e, a):
        kv_loop(VALUES, e * 2 * n_chunks, 2 * n_chunks, weigh_values)
        pair = pl.ds(2 * e, 2)
        acc_v[pair] = acc_v[pair] / jnp.sum(l_v[pair], axis=-1, keepdims=True)
        for slab in range(4):
            for i in range(3):
                a = a + project(4 * e + slab, i)
        return a

    a = lax.fori_loop(0, n_groups // 2, pair_body, jnp.zeros((8, d_model), f32))

    columns = {
        slab: jnp.broadcast_to(head_out(slab, 3).astype(dtype).astype(f32), (128, _DH)).T
        for slab in (6, 7)
    }
    for slabs in ((0, 1, 2, 3), (4, 5)):
        for slab in slabs:
            advance(WO_LAST, slab)
        for slab in slabs:
            a = a + project(slab, 3)
    a = jnp.where(lax.broadcasted_iota(jnp.int32, a.shape, 0) == 0, a, 0.0)
    for slab, column in columns.items():
        advance(WO_LAST, slab)
        w = wo_v[slab, pl.ds(3 * _DH, _DH)].astype(f32)
        a = a + jnp.concatenate(
            [(w[:, c:c + 128] * column).reshape(_DH // 8, 8, 128).sum(axis=0)
             for c in range(0, d_model, 128)], axis=1)
    o_ref[0] = (gate * jnp.sum(a, axis=0, keepdims=True) + b).astype(o_ref.dtype)


@jax.jit
def pallas_gated_mix__sliding_block_cached__swiglu_ffn__decode_kernel(
    A_x: jax.Array,
    A_k_cache: jax.Array,
    A_v_cache: jax.Array,
    A_wq: jax.Array,
    A_wo: jax.Array,
    B_x: jax.Array,
    B_w_gate: jax.Array,
    B_w_up: jax.Array,
    B_w_down: jax.Array,
    gate_w: jax.Array,
):
    del B_x
    d_model, d_ff = B_w_gate.shape
    seq = A_k_cache.shape[2]
    window = min(4096, max(256, seq // 4))
    dtype = A_x.dtype
    assert A_x.shape == (1, 1, 512) and A_k_cache.shape == (1, _HQ, seq, _DH)
    assert d_ff % 32 == 0 and d_ff // 32 >= _HQ and (seq - window) % 64 == 0
    n_groups = _HQ // 8
    wq_shape = (8, d_model // 8, _HQ * _DH)
    wo_shape = (8, _HQ * _DH // 8, d_model)
    ffn_shape = (2, d_ff // 2, d_model)
    gw_shape = (d_model // 128, 128)
    stat = pltpu.VMEM((n_groups, 8, 128), jnp.float32)

    return pl.pallas_call(
        functools.partial(_kernel, window=window),
        out_shape=jax.ShapeDtypeStruct(A_x.shape, dtype),
        in_specs=[pl.BlockSpec(memory_space=pltpu.HBM)] * 9,
        scratch_shapes=[
            pltpu.VMEM(A_x.shape, dtype),
            pltpu.VMEM(gw_shape, dtype),
            pltpu.VMEM(wq_shape, dtype),
            pltpu.VMEM(wo_shape, dtype),
            pltpu.VMEM(ffn_shape, dtype),
            pltpu.VMEM(ffn_shape, dtype),
            pltpu.VMEM(ffn_shape, dtype),
            pltpu.VMEM((_RING, 8, 128, _DH), dtype),
            stat,
            pltpu.VMEM((n_groups * window // 128, 8, 128), jnp.float32),
            stat,
            stat,
            stat,
            pltpu.SemaphoreType.DMA((_NSEM,)),
            pltpu.SemaphoreType.DMA((1,)),
        ],
        compiler_params=pltpu.CompilerParams(
            vmem_limit_bytes=32 * 2**20,
            disable_bounds_checks=True,
            disable_semaphore_checks=True,
        ),
    )(
        A_x,
        A_k_cache.reshape(n_groups, 8, seq, _DH),
        A_v_cache.reshape(n_groups, 8, seq, _DH),
        A_wq.reshape(wq_shape),
        A_wo.reshape(wo_shape),
        B_w_gate.T.reshape(ffn_shape),
        B_w_up.T.reshape(ffn_shape),
        B_w_down.reshape(ffn_shape),
        gate_w.reshape(gw_shape),
    )
```
